```python
import os as _os
_os.environ.setdefault("JAX_PLATFORMS", "cpu")
import jax
import jax.numpy as jnp

def _softmax(x, axis=-1):
    return jax.nn.softmax(x, axis=axis)
def _gelu(x):
    return jax.nn.gelu(x, approximate=True)
def _silu(x):
    return jax.nn.silu(x)
def _sigmoid(x):
    return jax.nn.sigmoid(x)
def _layernorm(x, axis=-1, eps=1e-5):
    m = jnp.mean(x, axis=axis, keepdims=True)
    v = jnp.var(x, axis=axis, keepdims=True)
    return (x - m) / jnp.sqrt(v + eps)
def _scatter_add(tgt, idx, src, axis=0):
    return tgt.at[idx].add(src)
def _segment_sum(src, seg, n):
    return jax.ops.segment_sum(src, seg, n)
class _Rng:
    def __init__(self, key):
        self._k = key
    def _next(self):
        self._k, sub = jax.random.split(self._k)
        return sub
    def normal(self, shape):
        return jax.random.normal(self._next(), shape, dtype=jnp.bfloat16)
    def randint(self, lo, hi, shape):
        return jax.random.randint(self._next(), shape, lo, hi, dtype=jnp.int32)
    def uniform(self, shape, lo=0.0, hi=1.0):
        return jax.random.uniform(self._next(), shape, jnp.bfloat16, lo, hi)
    def permutation(self, n):
        return jax.random.permutation(self._next(), n)


kernel_name = 'parallel_sum__softmax_full_mha__swiglu_ffn__prompt'

def setup_inputs():
    _rng = _Rng(jax.random.key(int.from_bytes(__import__("os").urandom(4), "little")))
    _w = (lambda a: (lambda t: t.astype(jnp.bfloat16) if jnp.issubdtype(t.dtype, jnp.floating) else t)(jnp.asarray(a)))
    def _A_setup():
        B, S, D = 1, 2048, 640
        return {
            "x": _w((lambda *s: _rng.normal(s) * 0.05)(B, S, D)),
            "wqkv": _w((lambda *s: _rng.normal(s) * 0.1)(D, 3 * D)),
            "wo": _w((lambda *s: _rng.normal(s) * 0.05)(D, D)),
        }
    _A_in = _A_setup()

    def _B_setup():
        B, S, D, F = 1, 2048, 640, 1536
        return {
            "x": _w((lambda *s: _rng.normal(s) * 0.05)(B, S, D)),
            "w_gate": _w((lambda *s: _rng.normal(s) * 0.05)(D, F)),
            "w_up": _w((lambda *s: _rng.normal(s) * 0.05)(D, F)),
            "w_down": _w((lambda *s: _rng.normal(s) * 0.05)(F, D)),
        }
    _B_in = _B_setup()

    return {
        "A_x": _A_in["x"],
        "A_wqkv": _A_in["wqkv"],
        "A_wo": _A_in["wo"],
        "B_x": _B_in["x"],
        "B_w_gate": _B_in["w_gate"],
        "B_w_up": _B_in["w_up"],
        "B_w_down": _B_in["w_down"],
    }

def reference(A_x, A_wqkv, A_wo, B_x, B_w_gate, B_w_up, B_w_down):
    def _A_ref(x, wqkv, wo):
        B, S, D = x.shape
        H = 32; Dh = D // H
        qkv = (lambda x, *d: x.transpose(*d))((x @ wqkv).reshape(B, S, 3, H, Dh), 2, 0, 3, 1, 4)
        q, k, v = qkv[0], qkv[1], qkv[2]
        scale = Dh ** -0.5
        scores = jnp.einsum("bhqd,bhkd->bhqk", q, k) * scale
        p = _softmax(scores, axis=-1)
        o = jnp.einsum("bhqk,bhkd->bhqd", p, v)
        return (lambda x, *d: x.transpose(*d))(o, 0, 2, 1, 3).reshape(B, S, D) @ wo

    def _B_ref(x, w_gate, w_up, w_down):
        g = _silu(x @ w_gate)
        u = x @ w_up
        return (g * u) @ w_down

    x = A_x
    xn = _layernorm(x, axis=-1)
    return x + _A_ref(xn, A_wqkv, A_wo) + _B_ref(xn, B_w_gate, B_w_up, B_w_down)
```

```python
import functools
import math

import jax
import jax.numpy as jnp
from jax import lax
from jax.experimental import pallas as pl
from jax.experimental.pallas import tpu as pltpu

S = 2048
D = 640
H = 32
DH = 20
F = 1536
EPS = 1e-5
LANES = 128
VROWS = 24
STRADDLE = (6, 12, 19, 25)
EXTRA_OFF = (0, 24, 44, 68)
NKB = 6

TQ = 512
TK = 128
TM = 256
TN = 256
LAG = 1
ZF0 = 12
ZF1 = 14
ZSTEP = 3
G1 = 3
WV_LATE = 0
UNROLL_B = 2


def _head_block(h):
    if h in STRADDLE:
        return 5, EXTRA_OFF[STRADDLE.index(h)]
    return (DH * h) // LANES, (DH * h) % LANES


def _pack(x):
    return pltpu.bitcast(x, jnp.uint32)


def _unpack(x):
    return pltpu.bitcast(x, jnp.bfloat16)


def _kernel(x_hbm, wqkv_hbm, wo_hbm, wg_hbm, wu_hbm, wd_hbm, o_hbm,
            x_ref, wqkv_ref, wo_ref, wg_ref, wu_ref, wd_ref, o_ref,
            wt_ref, xn_ref, k_ref, qm_ref, vt_ref, s_ref, m_ref, ot_ref,
            x_sem, w_sem, o_sem):
    f32 = jnp.float32
    bf16 = jnp.bfloat16
    qscale = (DH ** -0.5) * math.log2(math.e)
    NQB = S // TQ
    NIT = H // 2
    NB = 2 * NQB
    NRB = S // TM

    def x_copy(i):
        return pltpu.make_async_copy(x_hbm.at[pl.ds(i * TM, TM), :], x_ref.at[pl.ds(i * TM, TM), :], x_sem.at[i])

    def wqkv_copy(part):
        cols = pl.ds(part * D, D)
        return pltpu.make_async_copy(wqkv_hbm.at[:, cols], wqkv_ref.at[:, cols], w_sem.at[part])

    late = [(wg_hbm, wg_ref), (wu_hbm, wu_ref), (wd_hbm, wd_ref), (wo_hbm, wo_ref)]
    late_copies = [pltpu.make_async_copy(s, d, w_sem.at[3 + j]) for j, (s, d) in enumerate(late)]

    x_copy(0).start()
    wqkv_copy(1).start()
    for i in range(1, NRB):
        x_copy(i).start()
    wqkv_copy(0).start()
    wqkv_copy(2).start()

    def zero_fill(h0, h1):
        for h in range(h0, h1):
            qm_ref[h] = jnp.zeros(qm_ref.shape[1:], jnp.uint32)

    def layernorm(i):
        r0 = i * TM
        x = x_ref[r0:r0 + TM, :].astype(f32)
        mu = jnp.mean(x, axis=-1, keepdims=True)
        xc = x - mu
        var = jnp.mean(xc * xc, axis=-1, keepdims=True)
        xn_ref[r0:r0 + TM, :] = (xc * lax.rsqrt(var + EPS)).astype(bf16)

    def kproj(i):
        r0 = i * TM
        kk = jnp.dot(xn_ref[r0:r0 + TM, :], wqkv_ref[:, D:2 * D], preferred_element_type=f32).astype(bf16)
        for b in range(D // LANES):
            k_ref[b, r0 // 2:(r0 + TM) // 2, :] = _pack(kk[:, b * LANES:(b + 1) * LANES])

    def transpose_w(cb):
        wblk = wqkv_ref[:, cb * LANES:(cb + 1) * LANES].astype(f32)
        wt_ref[cb * LANES:(cb + 1) * LANES, :] = wblk.T

    zero_fill(0, ZF0)
    x_copy(0).wait()
    layernorm(0)
    zero_fill(ZF0, ZF1)
    wqkv_copy(1).wait()
    for i in range(1, G1 + 1):
        x_copy(i).wait()
    zpos = ZF1
    for i in range(G1):
        kproj(i)
        layernorm(i + 1)
        for cb in range(5, 10):
            if (cb - 5) % G1 == i:
                transpose_w(cb)
        z1 = min(H, zpos + ZSTEP)
        zero_fill(zpos, z1)
        zpos = z1
    for i in range(G1 + 1, NRB):
        x_copy(i).wait()
    wqkv_copy(0).wait()
    if not WV_LATE:
        wqkv_copy(2).wait()
    rest = list(range(0, 5)) + ([] if WV_LATE else list(range(10, 15)))
    nrest = NRB - G1
    for i in range(G1, NRB):
        kproj(i)
        if i + 1 < NRB:
            layernorm(i + 1)
        for j, cb in enumerate(rest):
            if j % nrest == i - G1:
                transpose_w(cb)
        z1 = min(H, zpos + ZSTEP)
        zero_fill(zpos, z1)
        zpos = z1
    assert zpos == H
    if WV_LATE:
        wqkv_copy(2).wait()
        for cb in range(10, 15):
            transpose_w(cb)
    for c in late_copies:
        c.start()

    rows128w = lax.broadcasted_iota(jnp.int32, (LANES, D), 0)
    wkx = jnp.zeros((LANES, D), f32)
    for h, off in zip(STRADDLE, EXTRA_OFF):
        start = D + DH * h - off
        wkx = jnp.where((rows128w >= off) & (rows128w < off + DH), wt_ref[start:start + LANES, :], wkx)
    wt_ref[3 * D:3 * D + LANES, :] = wkx

    def proj_body(i, carry):
        c0 = pl.multiple_of(i * TN, TN)
        xn = xn_ref[pl.ds(c0, TN), :]
        nt = (((1,), (1,)), ((), ()))
        kx = lax.dot_general(xn, wt_ref[3 * D:3 * D + LANES, :].astype(bf16), nt, preferred_element_type=f32)
        k_ref[NKB - 1, pl.ds(pl.multiple_of(i * (TN // 2), TN // 2), TN // 2), :] = _pack(kx.astype(bf16))
        qT = lax.dot_general(wt_ref[0:D, :], xn, nt, preferred_element_type=f32) * qscale
        for h in range(H):
            blk, off = _head_block(h)
            lo = (off // 16) * 16
            hi = -(-(off + DH) // 16) * 16
            start = DH * h - off
            win = qT[start + lo:start + hi]
            rr = lax.broadcasted_iota(jnp.int32, (hi - lo, TN), 0) + lo
            qm = jnp.where((rr >= off) & (rr < off + DH), win, 0.0)
            qm_ref[h, lo // 2:hi // 2, pl.ds(c0, TN)] = _pack(qm.astype(bf16))
        vT = lax.dot_general(wt_ref[2 * D:3 * D, :], xn, nt, preferred_element_type=f32)
        rows24 = lax.broadcasted_iota(jnp.int32, (VROWS, TN), 0)
        for h in range(H):
            vs = DH * h - (4 if h % 2 else 0)
            ones_row = 0 if h % 2 else DH
            vt_ref[h, :, pl.ds(c0, TN)] = jnp.where(rows24 == ones_row, 1.0, vT[vs:vs + VROWS])
        return carry

    lax.fori_loop(0, S // TN, proj_body, 0, unroll=UNROLL_B)

    def kblock(h):
        b = (DH * h) // LANES
        is_str = (h == 6) | (h == 12) | (h == 19) | (h == 25)
        return jnp.where(is_str, NKB - 1, b)

    def unit_of(it, u):
        it2 = jnp.minimum(it + u // NB, NIT - 1)
        u2 = u % NB
        h = 2 * it2 + u2 // NQB
        return (h, (u2 % NQB) * TQ, u2 >= NQB)

    NC = S // TK
    rows8 = lax.broadcasted_iota(jnp.int32, (8, TQ), 0)

    class AState:
        def __init__(self, unit, slot):
            self.h, self.q, self.odd = unit
            self.kb = kblock(self.h)
            self.slot = slot
            self.macc = None

    class BState:
        def __init__(self, unit, slot):
            self.h, self.q, self.odd = unit
            self.slot = slot
            self.acc = None
            self.m = None

    def a_item(st, c):
        k0, k1 = c * TK, (c + 1) * TK
        kc = _unpack(k_ref[st.kb, k0 // 2:k1 // 2, :])
        qc = _unpack(qm_ref[st.h, :, st.q:st.q + TQ])
        s = jnp.dot(kc, qc, preferred_element_type=f32)
        s_ref[st.slot, k0:k1, :] = s
        cm = jnp.max(s.reshape(TK // 8, 8, TQ), axis=0)
        st.macc = cm if st.macc is None else jnp.maximum(st.macc, cm)
        if c == NC - 1:
            mx = jnp.max(st.macc, axis=0, keepdims=True)
            m_ref[st.slot] = jnp.broadcast_to(mx, (8, TQ))

    def b_item(st, c, r0):
        if st.m is None:
            st.m = m_ref[st.slot]
        ks = slice(c * TK, (c + 1) * TK)
        sv = s_ref[st.slot, ks, :].reshape(TK // 8, 8, TQ)
        p = jnp.exp2(sv - st.m[None]).reshape(TK, TQ).astype(bf16)
        pv = jnp.dot(vt_ref[st.h, :, ks], p, preferred_element_type=f32)
        st.acc = pv if st.acc is None else st.acc + pv
        if c == NC - 1:
            lrow = 0 if st.odd else DH
            res = st.acc * (1.0 / st.acc[lrow:lrow + 1, :])
            qq = st.q
            if not st.odd:
                ot_ref[pl.ds(r0, VROWS), qq:qq + TQ] = res
            else:
                r1 = pl.multiple_of(r0 + 16, 8)
                ev = ot_ref[pl.ds(r1, 8), qq:qq + TQ]
                mid = jnp.where(rows8 < 4, ev, res[0:8])
                ot_ref[pl.ds(r1, VROWS), qq:qq + TQ] = jnp.concatenate([mid, res[8:]], axis=0)

    st0 = AState(unit_of(jnp.int32(0), 0), 0)
    for c in range(NC):
        a_item(st0, c)

    b_pos = []
    for u in range(NB):
        lo = u * NC + (LAG if u > 0 else 0)
        hi = min((u + 1) * NC + LAG, NB * NC)
        for j in range(NC):
            b_pos.append((lo + (j * (hi - lo)) // NC, u, j))

    def attn_body(it, carry):
        r0 = pl.multiple_of(it * (2 * DH), 8)
        a_states = [AState(unit_of(it, u + 1), (u + 1) % 2) for u in range(NB)]
        b_states = [BState(unit_of(it, u), u % 2) for u in range(NB)]
        bi = 0
        for t in range(NB * NC):
            a_item(a_states[t // NC], t % NC)
            while bi < len(b_pos) and b_pos[bi][0] <= t:
                _, u, j = b_pos[bi]
                b_item(b_states[u], j, r0)
                bi += 1
        return carry

    lax.fori_loop(0, NIT, attn_body, 0)

    for c in late_copies:
        c.wait()

    def o_copy(i):
        r0 = pl.multiple_of(i * TM, TM)
        return pltpu.make_async_copy(o_ref.at[pl.ds(r0, TM), :], o_hbm.at[pl.ds(r0, TM), :], o_sem.at[i])

    def out_body(i, carry):
        r0 = pl.multiple_of(i * TM, TM)
        xn = xn_ref[pl.ds(r0, TM), :]
        g = jnp.dot(xn, wg_ref[...], preferred_element_type=f32)
        u = jnp.dot(xn, wu_ref[...], preferred_element_type=f32)
        hh = (g * (1.0 / (1.0 + jnp.exp(-g))) * u).astype(bf16)
        y = jnp.dot(hh, wd_ref[...], preferred_element_type=f32)
        o = ot_ref[:, pl.ds(r0, TM)].T.astype(bf16)
        y = y + jnp.dot(o, wo_ref[...], preferred_element_type=f32)
        o_ref[pl.ds(r0, TM), :] = (x_ref[pl.ds(r0, TM), :].astype(f32) + y).astype(o_ref.dtype)
        o_copy(i).start()
        return carry

    lax.fori_loop(0, NRB, out_body, 0)
    for i in range(NRB):
        o_copy(i).wait()


@jax.jit
def pallas_parallel_sum__softmax_full_mha__swiglu_ffn__prompt_kernel(
        A_x, A_wqkv, A_wo, B_x, B_w_gate, B_w_up, B_w_down):
    x = A_x.reshape(S, D)
    bf16 = jnp.bfloat16
    out = pl.pallas_call(
        _kernel,
        out_shape=jax.ShapeDtypeStruct((S, D), A_x.dtype),
        in_specs=[pl.BlockSpec(memory_space=pl.ANY)] * 6,
        out_specs=pl.BlockSpec(memory_space=pl.ANY),
        scratch_shapes=[
            pltpu.VMEM((S, D), bf16),
            pltpu.VMEM((D, 3 * D), bf16),
            pltpu.VMEM((D, D), bf16),
            pltpu.VMEM((D, F), bf16),
            pltpu.VMEM((D, F), bf16),
            pltpu.VMEM((F, D), bf16),
            pltpu.VMEM((S, D), bf16),
            pltpu.VMEM((3 * D + LANES, D), jnp.float32),
            pltpu.VMEM((S, D), bf16),
            pltpu.VMEM((NKB, S // 2, LANES), jnp.uint32),
            pltpu.VMEM((H, LANES // 2, S), jnp.uint32),
            pltpu.VMEM((H, VROWS, S), jnp.float32),
            pltpu.VMEM((2, S, TQ), jnp.float32),
            pltpu.VMEM((2, 8, TQ), jnp.float32),
            pltpu.VMEM((D, S), jnp.float32),
            pltpu.SemaphoreType.DMA((S // TM,)),
            pltpu.SemaphoreType.DMA((7,)),
            pltpu.SemaphoreType.DMA((S // TM,)),
        ],
        compiler_params=pltpu.CompilerParams(vmem_limit_bytes=110 * 2**20),
    )(x, A_wqkv, A_wo, B_w_gate, B_w_up, B_w_down)
    return out.reshape(1, S, D)
```

```python
import functools
import math

import jax
import jax.numpy as jnp
from jax import lax
from jax.experimental import pallas as pl
from jax.experimental.pallas import tpu as pltpu

S = 2048
D = 640
H = 32
DH = 20
F = 1536
EPS = 1e-5
LANES = 128
VROWS = 24
STRADDLE = (6, 12, 19, 25)
NDB = D // LANES
NKB = NDB + len(STRADDLE)

TQ = 512
TK = 128
TX = 256
TA = 64
TN = 256
TM = 256
LAG = 1
G1 = 2
G2 = 5
X_LATE_AT = 4
ZF0 = 16


def _pack(x):
    return pltpu.bitcast(x, jnp.uint32)


def _unpack(x):
    return pltpu.bitcast(x, jnp.bfloat16)


def _head_bands(h):
    g0, g1 = DH * h, DH * (h + 1)
    if h in STRADDLE:
        mid = (g1 // LANES) * LANES
        return [(g0, mid), (mid, g1)]
    return [(g0, g1)]


def _kernel(x_hbm, wqkv_hbm, wo_hbm, wg_hbm, wu_hbm, wd_hbm, o_hbm,
            x_ref, wqkv_ref, wo_ref, wg_ref, wu_ref, wd_ref, o_ref,
            wt_ref, xn_ref, k_ref, qm_ref, vt_ref, s_ref, m_ref, ot_ref,
            x_sem, w_sem, o_sem):
    f32 = jnp.float32
    bf16 = jnp.bfloat16
    qscale = (DH ** -0.5) * math.log2(math.e)
    NQB = S // TQ
    NIT = H // 2
    NB = 2 * NQB
    NXB = S // TX
    NRB = S // TM
    NC = S // TK

    def x_copy(i):
        rows = pl.ds(i * TX, TX)
        return pltpu.make_async_copy(x_hbm.at[rows, :], x_ref.at[rows, :], x_sem.at[i])

    def wqkv_copy(part):
        cols = pl.ds(part * D, D)
        return pltpu.make_async_copy(wqkv_hbm.at[:, cols], wqkv_ref.at[:, cols], w_sem.at[part])

    late = [(wg_hbm, wg_ref), (wu_hbm, wu_ref), (wd_hbm, wd_ref), (wo_hbm, wo_ref)]
    late_copies = [pltpu.make_async_copy(s, d, w_sem.at[3 + j]) for j, (s, d) in enumerate(late)]

    def start_x(lo, hi):
        for i in range(lo, hi):
            x_copy(i).start()

    def wait_x(lo, hi):
        for i in range(lo, hi):
            x_copy(i).wait()

    x_copy(0).start()
    wqkv_copy(1).start()
    start_x(1, G1)

    low_lanes = lax.broadcasted_iota(jnp.int32, (TA // 2, LANES), 1) < LANES // 2

    def ln(p):
        r0 = p * TA
        x = x_ref[r0:r0 + TA, :].astype(f32)
        mu = jnp.mean(x, axis=-1, keepdims=True)
        xc = x - mu
        var = jnp.mean(xc * xc, axis=-1, keepdims=True)
        xn_ref[r0:r0 + TA, :] = (xc * lax.rsqrt(var + EPS)).astype(bf16)

    def kproj(p):
        r0 = p * TA
        xn = xn_ref[r0:r0 + TA, :]
        kk = jnp.dot(xn, wqkv_ref[:, D:2 * D], preferred_element_type=f32).astype(bf16)
        kb = [_pack(kk[:, b * LANES:(b + 1) * LANES]) for b in range(NDB)]
        for b in range(NDB):
            k_ref[b, r0 // 2:(r0 + TA) // 2, :] = kb[b]
        for b in range(NDB - 1):
            k_ref[NDB + b, r0 // 2:(r0 + TA) // 2, :] = jnp.where(low_lanes, kb[b + 1], kb[b])

    def transpose_w(j):
        cb = j if j < NDB else j + NDB
        wblk = wqkv_ref[:, cb * LANES:(cb + 1) * LANES].astype(f32).T
        wt_ref[j * LANES // 2:(j + 1) * LANES // 2, :] = _pack(wblk.astype(bf16))

    PB = TX // TA
    NP = S // TA

    def run_pieces(ln_lo, ln_hi, kp_lo, kp_hi, extras=(), at=None):
        extras = list(extras)
        at = at or {}
        li, ki = ln_lo, kp_lo
        step = 0
        while li < ln_hi or ki < kp_hi:
            if ki < kp_hi and ki < li:
                kproj(ki)
                ki += 1
                step += 1
                for e in at.get(step, ()):
                    e()
                for j, e in enumerate(extras):
                    if (j * max(kp_hi - kp_lo - 2, 1)) // len(extras) == step - 1:
                        e()
            if li < ln_hi:
                ln(li)
                li += 1

    def zero_s(j, carry):
        r = pl.multiple_of(j * TK, TK)
        s_ref[1, pl.ds(r, TK), :] = jnp.zeros((TK, TQ), f32)
        return carry

    def zero_q(h, carry):
        qm_ref[h] = jnp.zeros(qm_ref.shape[1:], jnp.uint32)
        return carry

    lax.fori_loop(0, NC, zero_s, 0)
    m_ref[1] = jnp.zeros(m_ref.shape[1:], f32)
    ot_ref[16:24, S - TQ:S] = jnp.zeros((8, TQ), f32)
    lax.fori_loop(0, ZF0, zero_q, 0)

    x_copy(0).wait()
    for p in range(PB):
        ln(p)
    wqkv_copy(1).wait()
    wait_x(1, G1)
    start_x(G1, G2)
    run_pieces(PB, G1 * PB, 0, G1 * PB - 1, at={X_LATE_AT: [functools.partial(start_x, G2, NXB)]})
    wait_x(G1, G2)
    wqkv_copy(0).start()
    wqkv_copy(2).start()
    run_pieces(G1 * PB, G2 * PB, G1 * PB - 1, G2 * PB - 1)
    wait_x(G2, NXB)
    wqkv_copy(0).wait()
    wqkv_copy(2).wait()
    for c in late_copies:
        c.start()
    run_pieces(G2 * PB, NP, G2 * PB - 1, NP,
               [functools.partial(transpose_w, j) for j in range(2 * NDB)])

    def proj_body(i, carry):
        c0 = pl.multiple_of(i * TN, TN)
        xn = xn_ref[pl.ds(c0, TN), :]
        nt = (((1,), (1,)), ((), ()))
        for h in range(ZF0, H):
            used = set()
            for a, b in _head_bands(h):
                used |= set(g % (LANES // 16) for g in range(a // 16, -(-b // 16)))
            for g in range(LANES // 16):
                if g not in used:
                    qm_ref[h, g * 8:(g + 1) * 8, pl.ds(c0, TN)] = jnp.zeros((8, TN), jnp.uint32)
        qT = lax.dot_general(_unpack(wt_ref[0:D // 2, :]), xn, nt,
                             preferred_element_type=f32) * qscale
        for h in range(H):
            for a, b in _head_bands(h):
                lo = (a // 16) * 16
                hi = -(-b // 16) * 16
                rr = lax.broadcasted_iota(jnp.int32, (hi - lo, TN), 0) + lo
                qm = jnp.where((rr >= a) & (rr < b), qT[lo:hi], 0.0)
                l0 = lo % LANES
                qm_ref[h, l0 // 2:(l0 + hi - lo) // 2, pl.ds(c0, TN)] = _pack(qm.astype(bf16))
        vT = lax.dot_general(_unpack(wt_ref[D // 2:D, :]), xn, nt, preferred_element_type=f32)
        rows24 = lax.broadcasted_iota(jnp.int32, (VROWS, TN), 0)
        for h in range(H):
            vs = DH * h - (4 if h % 2 else 0)
            ones_row = 0 if h % 2 else DH
            vt_ref[h, :, pl.ds(c0, TN)] = jnp.where(rows24 == ones_row, 1.0, vT[vs:vs + VROWS])
        return carry

    lax.fori_loop(0, S // TN, proj_body, 0, unroll=2)

    def kblock(h):
        b = (DH * h) // LANES
        is_str = (h == 6) | (h == 12) | (h == 19) | (h == 25)
        return jnp.where(is_str, NDB + b, b)

    def unit_of(it, u):
        pair = jnp.clip(it + u // NB, 0, NIT - 1)
        u2 = u % NB
        odd = u2 // NQB
        return 2 * pair + odd, (u2 % NQB) * TQ, odd == 1, pair

    rows8 = lax.broadcasted_iota(jnp.int32, (8, TQ), 0)

    class QKState:
        def __init__(self, unit, slot):
            self.h, self.q, _, _ = unit
            self.kb = kblock(self.h)
            self.slot = slot
            self.macc = None

    class PVState:
        def __init__(self, unit, slot):
            self.h, self.q, self.odd, self.pair = unit
            self.slot = slot
            self.acc = None
            self.m = None

    def qk_chunk(st, c):
        k0, k1 = c * TK, (c + 1) * TK
        kc = _unpack(k_ref[st.kb, k0 // 2:k1 // 2, :])
        qc = _unpack(qm_ref[st.h, :, st.q:st.q + TQ])
        s = jnp.dot(kc, qc, preferred_element_type=f32)
        s_ref[st.slot, k0:k1, :] = s
        cm = jnp.max(s.reshape(TK // 8, 8, TQ), axis=0)
        st.macc = cm if st.macc is None else jnp.maximum(st.macc, cm)
        if c == NC - 1:
            mx = jnp.max(st.macc, axis=0, keepdims=True)
            m_ref[st.slot] = jnp.broadcast_to(mx, (8, TQ))

    def pv_chunk(st, c):
        if st.m is None:
            st.m = m_ref[st.slot]
        ks = slice(c * TK, (c + 1) * TK)
        sv = s_ref[st.slot, ks, :].reshape(TK // 8, 8, TQ)
        p = jnp.exp2(sv - st.m[None]).reshape(TK, TQ).astype(bf16)
        pv = jnp.dot(vt_ref[st.h, :, ks], p, preferred_element_type=f32)
        st.acc = pv if st.acc is None else st.acc + pv
        if c == NC - 1:
            lrow = 0 if st.odd else DH
            res = st.acc * (1.0 / st.acc[lrow:lrow + 1, :])
            cols = slice(st.q, st.q + TQ)
            r0 = pl.multiple_of(st.pair * (2 * DH), 8)
            if not st.odd:
                ot_ref[pl.ds(r0, VROWS), cols] = res
            else:
                r1 = pl.multiple_of(r0 + 16, 8)
                even_tail = ot_ref[pl.ds(r1, 8), cols]
                mid = jnp.where(rows8 < 4, even_tail, res[0:8])
                ot_ref[pl.ds(r1, VROWS), cols] = jnp.concatenate([mid, res[8:]], axis=0)

    pv_pos = []
    for u in range(NB):
        lo = u * NC + (LAG if u > 0 else 0)
        hi = min((u + 1) * NC + LAG, NB * NC)
        for j in range(NC):
            pv_pos.append((lo + (j * (hi - lo)) // NC, u, j))

    def attn_body(it, carry):
        qk_states = [QKState(unit_of(it, u), u % 2) for u in range(NB)]
        pv_states = [PVState(unit_of(it, u - 1), (u - 1) % 2) for u in range(NB)]
        bi = 0
        for t in range(NB * NC):
            qk_chunk(qk_states[t // NC], t % NC)
            while bi < len(pv_pos) and pv_pos[bi][0] <= t:
                _, u, j = pv_pos[bi]
                pv_chunk(pv_states[u], j)
                bi += 1
        return carry

    lax.fori_loop(0, NIT, attn_body, 0)
    last = PVState(unit_of(jnp.int32(NIT - 1), NB - 1), (NB - 1) % 2)
    for c in range(NC):
        pv_chunk(last, c)

    for c in late_copies:
        c.wait()

    def o_copy(i):
        rows = pl.ds(pl.multiple_of(i * TM, TM), TM)
        return pltpu.make_async_copy(o_ref.at[rows, :], o_hbm.at[rows, :], o_sem.at[i])

    def out_body(i, carry):
        rows = pl.ds(pl.multiple_of(i * TM, TM), TM)
        xn = xn_ref[rows, :]
        g = jnp.dot(xn, wg_ref[...], preferred_element_type=f32)
        u = jnp.dot(xn, wu_ref[...], preferred_element_type=f32)
        hh = (g * (1.0 / (1.0 + jnp.exp(-g))) * u).astype(bf16)
        y = jnp.dot(hh, wd_ref[...], preferred_element_type=f32)
        o = ot_ref[:, rows].T.astype(bf16)
        y = y + jnp.dot(o, wo_ref[...], preferred_element_type=f32)
        o_ref[rows, :] = (x_ref[rows, :].astype(f32) + y).astype(o_ref.dtype)
        o_copy(i).start()
        return carry

    lax.fori_loop(0, NRB, out_body, 0)
    for i in range(NRB):
        o_copy(i).wait()


@jax.jit
def pallas_parallel_sum__softmax_full_mha__swiglu_ffn__prompt_kernel(
    A_x: jax.Array,
    A_wqkv: jax.Array,
    A_wo: jax.Array,
    B_x: jax.Array,
    B_w_gate: jax.Array,
    B_w_up: jax.Array,
    B_w_down: jax.Array,
):
    del B_x
    bf16 = jnp.bfloat16
    out = pl.pallas_call(
        _kernel,
        out_shape=jax.ShapeDtypeStruct((S, D), A_x.dtype),
        in_specs=[pl.BlockSpec(memory_space=pl.ANY)] * 6,
        out_specs=pl.BlockSpec(memory_space=pl.ANY),
        scratch_shapes=[
            pltpu.VMEM((S, D), bf16),
            pltpu.VMEM((D, 3 * D), bf16),
            pltpu.VMEM((D, D), bf16),
            pltpu.VMEM((D, F), bf16),
            pltpu.VMEM((D, F), bf16),
            pltpu.VMEM((F, D), bf16),
            pltpu.VMEM((S, D), bf16),
            pltpu.VMEM((D, D), jnp.uint32),
            pltpu.VMEM((S, D), bf16),
            pltpu.VMEM((NKB, S // 2, LANES), jnp.uint32),
            pltpu.VMEM((H, LANES // 2, S), jnp.uint32),
            pltpu.VMEM((H, VROWS, S), jnp.float32),
            pltpu.VMEM((2, S, TQ), jnp.float32),
            pltpu.VMEM((2, 8, TQ), jnp.float32),
            pltpu.VMEM((D, S), jnp.float32),
            pltpu.SemaphoreType.DMA((S // TX,)),
            pltpu.SemaphoreType.DMA((7,)),
            pltpu.SemaphoreType.DMA((S // TM,)),
        ],
        compiler_params=pltpu.CompilerParams(vmem_limit_bytes=100 * 2**20),
    )(A_x.reshape(S, D), A_wqkv, A_wo, B_w_gate, B_w_up, B_w_down)
    return out.reshape(1, S, D)
```

```python
import functools
import math

import jax
import jax.numpy as jnp
from jax import lax
from jax.experimental import pallas as pl
from jax.experimental.pallas import tpu as pltpu

S = 2048
D = 640
H = 32
DH = 20
F = 1536
EPS = 1e-5
LANES = 128
VROWS = 24
STRADDLE = (6, 12, 19, 25)
NDB = D // LANES
NKB = NDB + len(STRADDLE)
NIT = H // 2

TQ = 512
TK = 128
TA = 64
TN = 512
TF = S // NIT
TP = 128
LAG = 1
X_SPLITS = (0, 256, 512, 1280, 2048)
X_LATE_AT = 4
ZF0 = 12
FFN_UP_AT = 4
FFN_DOWN_AT = 40
PV_PER_PIECE = 2

SEM_WK, SEM_WQV, SEM_LATE, SEM_OUT, NSEM = 4, 5, 6, 7, 8


def _pack(x):
    return pltpu.bitcast(x, jnp.uint32)


def _unpack(x):
    return pltpu.bitcast(x, jnp.bfloat16)


def _head_bands(h):
    g0, g1 = DH * h, DH * (h + 1)
    if h in STRADDLE:
        mid = (g1 // LANES) * LANES
        return [(g0, mid), (mid, g1)]
    return [(g0, g1)]


def _kernel(x_hbm, wqkv_hbm, wo_hbm, wg_hbm, wu_hbm, wd_hbm, o_hbm,
            x_ref, wqkv_ref, wo_ref, wg_ref, wu_ref, wd_ref, o_ref,
            wt_ref, xn_ref, k_ref, qm_ref, vt_ref, s_ref, m_ref, ot_ref, hh_ref, y_ref,
            sem):
    f32 = jnp.float32
    bf16 = jnp.bfloat16
    qscale = (DH ** -0.5) * math.log2(math.e)
    NQB = S // TQ
    NB = 2 * NQB
    NC = S // TK

    def x_copy(g):
        rows = pl.ds(X_SPLITS[g], X_SPLITS[g + 1] - X_SPLITS[g])
        return pltpu.make_async_copy(x_hbm.at[rows, :], x_ref.at[rows, :], sem.at[g])

    def wqkv_copy(part):
        cols = pl.ds(part * D, D)
        return pltpu.make_async_copy(wqkv_hbm.at[:, cols], wqkv_ref.at[:, cols],
                                     sem.at[SEM_WK if part == 1 else SEM_WQV])

    late = [(wg_hbm, wg_ref), (wu_hbm, wu_ref), (wd_hbm, wd_ref), (wo_hbm, wo_ref)]
    late_copies = [pltpu.make_async_copy(s, d, sem.at[SEM_LATE]) for s, d in late]

    x_copy(0).start()
    wqkv_copy(1).start()
    x_copy(1).start()

    low_lanes = lax.broadcasted_iota(jnp.int32, (TA // 2, LANES), 1) < LANES // 2

    def ln(p):
        r0 = p * TA
        x = x_ref[r0:r0 + TA, :].astype(f32)
        mu = jnp.mean(x, axis=-1, keepdims=True)
        xc = x - mu
        var = jnp.mean(xc * xc, axis=-1, keepdims=True)
        xn_ref[r0:r0 + TA, :] = (xc * lax.rsqrt(var + EPS)).astype(bf16)

    def kproj(p):
        r0 = p * TA
        xn = xn_ref[r0:r0 + TA, :]
        kk = jnp.dot(xn, wqkv_ref[:, D:2 * D], preferred_element_type=f32).astype(bf16)
        kb = [_pack(kk[:, b * LANES:(b + 1) * LANES]) for b in range(NDB)]
        for b in range(NDB):
            k_ref[b, r0 // 2:(r0 + TA) // 2, :] = kb[b]
        for b in range(NDB - 1):
            k_ref[NDB + b, r0 // 2:(r0 + TA) // 2, :] = jnp.where(low_lanes, kb[b + 1], kb[b])

    def transpose_w(j):
        cb = j if j < NDB else j + NDB
        wblk = wqkv_ref[:, cb * LANES:(cb + 1) * LANES].astype(f32).T
        wt_ref[j * LANES // 2:(j + 1) * LANES // 2, :] = _pack(wblk.astype(bf16))

    def run_pieces(ln_lo, ln_hi, kp_lo, kp_hi, extras=(), at=None):
        extras = list(extras)
        at = at or {}
        li, ki = ln_lo, kp_lo
        step = 0
        while li < ln_hi or ki < kp_hi:
            if ki < kp_hi and ki < li:
                kproj(ki)
                ki += 1
                step += 1
                for e in at.get(step, ()):
                    e()
                for j, e in enumerate(extras):
                    if (j * max(kp_hi - kp_lo - 2, 1)) // len(extras) == step - 1:
                        e()
            if li < ln_hi:
                ln(li)
                li += 1

    def zero_s(j, carry):
        r = pl.multiple_of(j * TK, TK)
        s_ref[1, pl.ds(r, TK), :] = jnp.zeros((TK, TQ), f32)
        return carry

    def zero_q(h, carry):
        qm_ref[h] = jnp.zeros(qm_ref.shape[1:], jnp.uint32)
        return carry

    lax.fori_loop(0, NC, zero_s, 0)
    m_ref[1] = jnp.zeros(m_ref.shape[1:], f32)
    ot_ref[16:24, S - TQ:S] = jnp.zeros((8, TQ), f32)
    lax.fori_loop(0, ZF0, zero_q, 0)

    p1, p2, p3, p4 = (r // TA for r in X_SPLITS[1:])
    x_copy(0).wait()
    for p in range(p1):
        ln(p)
    wqkv_copy(1).wait()
    x_copy(1).wait()
    x_copy(2).start()
    run_pieces(p1, p2, 0, p2 - 1, at={X_LATE_AT: [x_copy(3).start]})
    x_copy(2).wait()
    wqkv_copy(0).start()
    wqkv_copy(2).start()
    run_pieces(p2, p3, p2 - 1, p3 - 1)
    x_copy(3).wait()
    wqkv_copy(0).wait()
    wqkv_copy(2).wait()
    for c in late_copies:
        c.start()
    run_pieces(p3, p4, p3 - 1, p4, [functools.partial(transpose_w, j) for j in range(2 * NDB)])

    def proj_body(i, carry):
        c0 = pl.multiple_of(i * TN, TN)
        xn = xn_ref[pl.ds(c0, TN), :]
        nt = (((1,), (1,)), ((), ()))
        for h in range(ZF0, H):
            used = set()
            for a, b in _head_bands(h):
                used |= set(g % (LANES // 16) for g in range(a // 16, -(-b // 16)))
            for g in range(LANES // 16):
                if g not in used:
                    qm_ref[h, g * 8:(g + 1) * 8, pl.ds(c0, TN)] = jnp.zeros((8, TN), jnp.uint32)
        qT = lax.dot_general(_unpack(wt_ref[0:D // 2, :]), xn, nt,
                             preferred_element_type=f32) * qscale
        for h in range(H):
            for a, b in _head_bands(h):
                lo = (a // 16) * 16
                hi = -(-b // 16) * 16
                rr = lax.broadcasted_iota(jnp.int32, (hi - lo, TN), 0) + lo
                qm = jnp.where((rr >= a) & (rr < b), qT[lo:hi], 0.0)
                l0 = lo % LANES
                qm_ref[h, l0 // 2:(l0 + hi - lo) // 2, pl.ds(c0, TN)] = _pack(qm.astype(bf16))
        vT = lax.dot_general(_unpack(wt_ref[D // 2:D, :]), xn, nt, preferred_element_type=f32)
        rows24 = lax.broadcasted_iota(jnp.int32, (VROWS, TN), 0)
        for h in range(H):
            vs = DH * h - (4 if h % 2 else 0)
            ones_row = 0 if h % 2 else DH
            vt_ref[h, :, pl.ds(c0, TN)] = jnp.where(rows24 == ones_row, 1.0, vT[vs:vs + VROWS])
        return carry

    lax.fori_loop(0, S // TN, proj_body, 0)

    def kblock(h):
        b = (DH * h) // LANES
        is_str = (h == 6) | (h == 12) | (h == 19) | (h == 25)
        return jnp.where(is_str, NDB + b, b)

    def unit_of(it, u):
        pair = jnp.clip(it + u // NB, 0, NIT - 1)
        u2 = u % NB
        odd = u2 // NQB
        return 2 * pair + odd, (u2 % NQB) * TQ, odd == 1, pair

    rows8 = lax.broadcasted_iota(jnp.int32, (8, TQ), 0)

    class QKState:
        def __init__(self, unit, slot):
            self.h, self.q, _, _ = unit
            self.kb = kblock(self.h)
            self.slot = slot
            self.macc = None

    class PVState:
        def __init__(self, unit, slot):
            self.h, self.q, self.odd, self.pair = unit
            self.slot = slot
            self.acc = None
            self.m = None

    def qk_chunk(st, c):
        k0, k1 = c * TK, (c + 1) * TK
        kc = _unpack(k_ref[st.kb, k0 // 2:k1 // 2, :])
        qc = _unpack(qm_ref[st.h, :, st.q:st.q + TQ])
        s = jnp.dot(kc, qc, preferred_element_type=f32)
        s_ref[st.slot, k0:k1, :] = s
        cm = jnp.max(s.reshape(TK // 8, 8, TQ), axis=0)
        st.macc = cm if st.macc is None else jnp.maximum(st.macc, cm)
        if c == NC - 1:
            mx = jnp.max(st.macc, axis=0, keepdims=True)
            m_ref[st.slot] = jnp.broadcast_to(mx, (8, TQ))

    def pv_chunk(st, c):
        if st.m is None:
            st.m = m_ref[st.slot]
        ks = slice(c * TK, (c + 1) * TK)
        sv = s_ref[st.slot, ks, :].reshape(TK // 8, 8, TQ)
        p = jnp.exp2(sv - st.m[None]).reshape(TK, TQ).astype(bf16)
        pv = jnp.dot(vt_ref[st.h, :, ks], p, preferred_element_type=f32)
        st.acc = pv if st.acc is None else st.acc + pv
        if c == NC - 1:
            lrow = 0 if st.odd else DH
            res = st.acc * (1.0 / st.acc[lrow:lrow + 1, :])
            cols = slice(st.q, st.q + TQ)
            r0 = pl.multiple_of(st.pair * (2 * DH), 8)
            if not st.odd:
                ot_ref[pl.ds(r0, VROWS), cols] = res
            else:
                r1 = pl.multiple_of(r0 + 16, 8)
                even_tail = ot_ref[pl.ds(r1, 8), cols]
                mid = jnp.where(rows8 < 4, even_tail, res[0:8])
                ot_ref[pl.ds(r1, VROWS), cols] = jnp.concatenate([mid, res[8:]], axis=0)

    def ffn_up(it):
        rows = pl.ds(pl.multiple_of(it * TF, TF), TF)
        xn = xn_ref[rows, :]
        g = jnp.dot(xn, wg_ref[...], preferred_element_type=f32)
        u = jnp.dot(xn, wu_ref[...], preferred_element_type=f32)
        hh_ref[...] = _pack((g * (1.0 / (1.0 + jnp.exp(-g))) * u).astype(bf16))

    def ffn_down(it):
        rows = pl.ds(pl.multiple_of(it * TF, TF), TF)
        y = jnp.dot(_unpack(hh_ref[...]), wd_ref[...], preferred_element_type=f32)
        y_ref[rows, :] = x_ref[rows, :].astype(f32) + y

    pv_pos = []
    for u in range(NB):
        lo = u * NC + (LAG if u > 0 else 0)
        hi = min((u + 1) * NC + LAG, NB * NC)
        for j in range(NC):
            pv_pos.append((lo + (j * (hi - lo)) // NC, u, j))

    def attn_body(it, carry):
        qk_states = [QKState(unit_of(it, u), u % 2) for u in range(NB)]
        pv_states = [PVState(unit_of(it, u - 1), (u - 1) % 2) for u in range(NB)]
        bi = 0
        for t in range(NB * NC):
            qk_chunk(qk_states[t // NC], t % NC)
            while bi < len(pv_pos) and pv_pos[bi][0] <= t:
                _, u, j = pv_pos[bi]
                pv_chunk(pv_states[u], j)
                bi += 1
            if t == FFN_UP_AT:
                ffn_up(it)
            if t == FFN_DOWN_AT:
                ffn_down(it)
        return carry

    for c in late_copies:
        c.wait()
    lax.fori_loop(0, NIT, attn_body, 0)

    assert (NC // PV_PER_PIECE) * TP <= S - TQ
    last = PVState(unit_of(jnp.int32(NIT - 1), NB - 1), (NB - 1) % 2)
    for j in range(S // TP):
        for c in range(min(NC, j * PV_PER_PIECE), min(NC, (j + 1) * PV_PER_PIECE)):
            pv_chunk(last, c)
        rows = slice(j * TP, (j + 1) * TP)
        o = ot_ref[:, rows].T.astype(bf16)
        y = y_ref[rows, :] + jnp.dot(o, wo_ref[...], preferred_element_type=f32)
        o_ref[rows, :] = y.astype(o_ref.dtype)
        drows = pl.ds(j * TP, TP)
        pltpu.make_async_copy(o_ref.at[drows, :], o_hbm.at[drows, :], sem.at[SEM_OUT]).start()
    pltpu.make_async_copy(o_ref, o_hbm, sem.at[SEM_OUT]).wait()


@jax.jit
def pallas_parallel_sum__softmax_full_mha__swiglu_ffn__prompt_kernel(
    A_x: jax.Array,
    A_wqkv: jax.Array,
    A_wo: jax.Array,
    B_x: jax.Array,
    B_w_gate: jax.Array,
    B_w_up: jax.Array,
    B_w_down: jax.Array,
):
    del B_x
    bf16 = jnp.bfloat16
    out = pl.pallas_call(
        _kernel,
        out_shape=jax.ShapeDtypeStruct((S, D), A_x.dtype),
        in_specs=[pl.BlockSpec(memory_space=pl.ANY)] * 6,
        out_specs=pl.BlockSpec(memory_space=pl.ANY),
        scratch_shapes=[
            pltpu.VMEM((S, D), bf16),
            pltpu.VMEM((D, 3 * D), bf16),
            pltpu.VMEM((D, D), bf16),
            pltpu.VMEM((D, F), bf16),
            pltpu.VMEM((D, F), bf16),
            pltpu.VMEM((F, D), bf16),
            pltpu.VMEM((S, D), bf16),
            pltpu.VMEM((D, D), jnp.uint32),
            pltpu.VMEM((S, D), bf16),
            pltpu.VMEM((NKB, S // 2, LANES), jnp.uint32),
            pltpu.VMEM((H, LANES // 2, S), jnp.uint32),
            pltpu.VMEM((H, VROWS, S), jnp.float32),
            pltpu.VMEM((2, S, TQ), jnp.float32),
            pltpu.VMEM((2, 8, TQ), jnp.float32),
            pltpu.VMEM((D, S), jnp.float32),
            pltpu.VMEM((TF // 2, F), jnp.uint32),
            pltpu.VMEM((S, D), jnp.float32),
            pltpu.SemaphoreType.DMA((NSEM,)),
        ],
        compiler_params=pltpu.CompilerParams(vmem_limit_bytes=100 * 2**20),
    )(A_x.reshape(S, D), A_wqkv, A_wo, B_w_gate, B_w_up, B_w_down)
    return out.reshape(1, S, D)
```

```python
import functools
import math

import jax
import jax.numpy as jnp
from jax import lax
from jax.experimental import pallas as pl
from jax.experimental.pallas import tpu as pltpu

S = 2048
D = 640
H = 32
DH = 20
F = 1536
EPS = 1e-5
LANES = 128
VROWS = 24
STRADDLE = (6, 12, 19, 25)
NDB = D // LANES
NKB = NDB + len(STRADDLE)
NIT = H // 2

TQ = 512
TK = 128
TA = 64
TN = 512
TF = S // NIT
TP = 128
LAG = 1
X_SPLITS = (0, 256, 512, 1280, 2048)
X_LATE_AT = 2
ZF0 = 12
FFN_UP_AT = 15
FFN_DOWN_AT = 127
PV_PER_PIECE = 2

SEM_WK, SEM_WQV, SEM_LATE, SEM_OUT, NSEM = 4, 5, 6, 7, 8


def _pack(x):
    return pltpu.bitcast(x, jnp.uint32)


def _unpack(x):
    return pltpu.bitcast(x, jnp.bfloat16)


def _head_bands(h):
    g0, g1 = DH * h, DH * (h + 1)
    if h in STRADDLE:
        mid = (g1 // LANES) * LANES
        return [(g0, mid), (mid, g1)]
    return [(g0, g1)]


def _kernel(x_hbm, wqkv_hbm, wo_hbm, wg_hbm, wu_hbm, wd_hbm, o_hbm,
            x_ref, wqkv_ref, wo_ref, wg_ref, wu_ref, wd_ref, o_ref,
            wt_ref, xn_ref, k_ref, qm_ref, vt_ref, s_ref, m_ref, ot_ref, hh_ref, y_ref,
            sem):
    f32 = jnp.float32
    bf16 = jnp.bfloat16
    qscale = (DH ** -0.5) * math.log2(math.e)
    NQB = S // TQ
    NB = 2 * NQB
    NC = S // TK

    def x_copy(g):
        rows = pl.ds(X_SPLITS[g], X_SPLITS[g + 1] - X_SPLITS[g])
        return pltpu.make_async_copy(x_hbm.at[rows, :], x_ref.at[rows, :], sem.at[g])

    def wqkv_copy(part):
        cols = pl.ds(part * D, D)
        return pltpu.make_async_copy(wqkv_hbm.at[:, cols], wqkv_ref.at[:, cols],
                                     sem.at[SEM_WK if part == 1 else SEM_WQV])

    late = [(wg_hbm, wg_ref), (wu_hbm, wu_ref), (wd_hbm, wd_ref), (wo_hbm, wo_ref)]
    late_copies = [pltpu.make_async_copy(s, d, sem.at[SEM_LATE]) for s, d in late]

    x_copy(0).start()
    wqkv_copy(1).start()
    x_copy(1).start()

    low_lanes = lax.broadcasted_iota(jnp.int32, (TA // 2, LANES), 1) < LANES // 2

    def ln(p):
        r0 = p * TA
        x = x_ref[r0:r0 + TA, :].astype(f32)
        mu = jnp.mean(x, axis=-1, keepdims=True)
        xc = x - mu
        var = jnp.mean(xc * xc, axis=-1, keepdims=True)
        xn_ref[r0:r0 + TA, :] = (xc * lax.rsqrt(var + EPS)).astype(bf16)

    def kproj(p):
        r0 = p * TA
        xn = xn_ref[r0:r0 + TA, :]
        kk = jnp.dot(xn, wqkv_ref[:, D:2 * D], preferred_element_type=f32).astype(bf16)
        kb = [_pack(kk[:, b * LANES:(b + 1) * LANES]) for b in range(NDB)]
        for b in range(NDB):
            k_ref[b, r0 // 2:(r0 + TA) // 2, :] = kb[b]
        for b in range(NDB - 1):
            k_ref[NDB + b, r0 // 2:(r0 + TA) // 2, :] = jnp.where(low_lanes, kb[b + 1], kb[b])

    def transpose_w(j):
        cb = j if j < NDB else j + NDB
        wblk = wqkv_ref[:, cb * LANES:(cb + 1) * LANES].astype(f32).T
        wt_ref[j * LANES // 2:(j + 1) * LANES // 2, :] = _pack(wblk.astype(bf16))

    def run_pieces(ln_lo, ln_hi, kp_lo, kp_hi, extras=(), at=None):
        extras = list(extras)
        at = at or {}
        li, ki = ln_lo, kp_lo
        step = 0
        fired = 0
        while li < ln_hi or ki < kp_hi:
            if ki < kp_hi and ki < li:
                kproj(ki)
                ki += 1
                step += 1
                for e in at.get(step, ()):
                    e()
                    fired += 1
                for j, e in enumerate(extras):
                    if (j * max(kp_hi - kp_lo - 2, 1)) // len(extras) == step - 1:
                        e()
                        fired += 1
            if li < ln_hi:
                ln(li)
                li += 1
        assert fired == len(extras) + sum(len(v) for v in at.values())

    def zero_s(j, carry):
        r = pl.multiple_of(j * TK, TK)
        s_ref[1, pl.ds(r, TK), :] = jnp.zeros((TK, TQ), f32)
        return carry

    def zero_q(h, carry):
        qm_ref[h] = jnp.zeros(qm_ref.shape[1:], jnp.uint32)
        return carry

    lax.fori_loop(0, NC, zero_s, 0)
    m_ref[1] = jnp.zeros(m_ref.shape[1:], f32)
    ot_ref[16:24, S - TQ:S] = jnp.zeros((8, TQ), f32)
    lax.fori_loop(0, ZF0, zero_q, 0)

    p1, p2, p3, p4 = (r // TA for r in X_SPLITS[1:])
    x_copy(0).wait()
    for p in range(p1):
        ln(p)
    wqkv_copy(1).wait()
    x_copy(1).wait()
    x_copy(2).start()
    run_pieces(p1, p2, 0, p2 - 1, at={X_LATE_AT: [x_copy(3).start]})
    x_copy(2).wait()
    wqkv_copy(0).start()
    wqkv_copy(2).start()
    run_pieces(p2, p3, p2 - 1, p3 - 1)
    x_copy(3).wait()
    wqkv_copy(0).wait()
    wqkv_copy(2).wait()
    for c in late_copies:
        c.start()
    run_pieces(p3, p4, p3 - 1, p4, [functools.partial(transpose_w, j) for j in range(2 * NDB)])

    def proj_body(i, carry):
        c0 = pl.multiple_of(i * TN, TN)
        xn = xn_ref[pl.ds(c0, TN), :]
        nt = (((1,), (1,)), ((), ()))
        for h in range(ZF0, H):
            used = set()
            for a, b in _head_bands(h):
                used |= set(g % (LANES // 16) for g in range(a // 16, -(-b // 16)))
            for g in range(LANES // 16):
                if g not in used:
                    qm_ref[h, g * 8:(g + 1) * 8, pl.ds(c0, TN)] = jnp.zeros((8, TN), jnp.uint32)
        qT = lax.dot_general(_unpack(wt_ref[0:D // 2, :]), xn, nt,
                             preferred_element_type=f32) * qscale
        for h in range(H):
            for a, b in _head_bands(h):
                lo = (a // 16) * 16
                hi = -(-b // 16) * 16
                rr = lax.broadcasted_iota(jnp.int32, (hi - lo, TN), 0) + lo
                qm = jnp.where((rr >= a) & (rr < b), qT[lo:hi], 0.0)
                l0 = lo % LANES
                qm_ref[h, l0 // 2:(l0 + hi - lo) // 2, pl.ds(c0, TN)] = _pack(qm.astype(bf16))
        vT = lax.dot_general(_unpack(wt_ref[D // 2:D, :]), xn, nt, preferred_element_type=f32)
        rows24 = lax.broadcasted_iota(jnp.int32, (VROWS, TN), 0)
        for h in range(H):
            vs = DH * h - (4 if h % 2 else 0)
            ones_row = 0 if h % 2 else DH
            vt_ref[h, :, pl.ds(c0, TN)] = jnp.where(rows24 == ones_row, 1.0, vT[vs:vs + VROWS])
        return carry

    lax.fori_loop(0, S // TN, proj_body, 0)

    def kblock(h):
        b = (DH * h) // LANES
        is_str = (h == 6) | (h == 12) | (h == 19) | (h == 25)
        return jnp.where(is_str, NDB + b, b)

    def unit_of(it, u):
        pair = jnp.clip(it + u // NB, 0, NIT - 1)
        u2 = u % NB
        odd = u2 // NQB
        return 2 * pair + odd, (u2 % NQB) * TQ, odd == 1, pair

    rows8 = lax.broadcasted_iota(jnp.int32, (8, TQ), 0)

    class QKState:
        def __init__(self, unit, slot):
            self.h, self.q, _, _ = unit
            self.kb = kblock(self.h)
            self.slot = slot
            self.macc = None

    class PVState:
        def __init__(self, unit, slot):
            self.h, self.q, self.odd, self.pair = unit
            self.slot = slot
            self.acc = None
            self.m = None

    def qk_chunk(st, c):
        k0, k1 = c * TK, (c + 1) * TK
        kc = _unpack(k_ref[st.kb, k0 // 2:k1 // 2, :])
        qc = _unpack(qm_ref[st.h, :, st.q:st.q + TQ])
        s = jnp.dot(kc, qc, preferred_element_type=f32)
        s_ref[st.slot, k0:k1, :] = s
        cm = jnp.max(s.reshape(TK // 8, 8, TQ), axis=0)
        st.macc = cm if st.macc is None else jnp.maximum(st.macc, cm)
        if c == NC - 1:
            mx = jnp.max(st.macc, axis=0, keepdims=True)
            m_ref[st.slot] = jnp.broadcast_to(mx, (8, TQ))

    def pv_chunk(st, c):
        if st.m is None:
            st.m = m_ref[st.slot]
        ks = slice(c * TK, (c + 1) * TK)
        sv = s_ref[st.slot, ks, :].reshape(TK // 8, 8, TQ)
        p = jnp.exp2(sv - st.m[None]).reshape(TK, TQ).astype(bf16)
        pv = jnp.dot(vt_ref[st.h, :, ks], p, preferred_element_type=f32)
        st.acc = pv if st.acc is None else st.acc + pv
        if c == NC - 1:
            lrow = 0 if st.odd else DH
            res = st.acc * (1.0 / st.acc[lrow:lrow + 1, :])
            cols = slice(st.q, st.q + TQ)
            r0 = pl.multiple_of(st.pair * (2 * DH), 8)
            if not st.odd:
                ot_ref[pl.ds(r0, VROWS), cols] = res
            else:
                r1 = pl.multiple_of(r0 + 16, 8)
                even_tail = ot_ref[pl.ds(r1, 8), cols]
                mid = jnp.where(rows8 < 4, even_tail, res[0:8])
                ot_ref[pl.ds(r1, VROWS), cols] = jnp.concatenate([mid, res[8:]], axis=0)

    def ffn_up(it):
        rows = pl.ds(pl.multiple_of(it * TF, TF), TF)
        xn = xn_ref[rows, :]
        g = jnp.dot(xn, wg_ref[...], preferred_element_type=f32)
        u = jnp.dot(xn, wu_ref[...], preferred_element_type=f32)
        hh_ref[...] = _pack((g * (1.0 / (1.0 + jnp.exp(-g))) * u).astype(bf16))

    def ffn_down(it):
        rows = pl.ds(pl.multiple_of(it * TF, TF), TF)
        y = jnp.dot(_unpack(hh_ref[...]), wd_ref[...], preferred_element_type=f32)
        y_ref[rows, :] = x_ref[rows, :].astype(f32) + y

    pv_pos = []
    for u in range(NB):
        lo = u * NC + (LAG if u > 0 else 0)
        hi = min((u + 1) * NC + LAG, NB * NC)
        for j in range(NC):
            pv_pos.append((lo + (j * (hi - lo)) // NC, u, j))

    def attn_body(it, carry):
        qk_states = [QKState(unit_of(it, u), u % 2) for u in range(NB)]
        pv_states = [PVState(unit_of(it, u - 1), (u - 1) % 2) for u in range(NB)]
        bi = 0
        for t in range(NB * NC):
            qk_chunk(qk_states[t // NC], t % NC)
            while bi < len(pv_pos) and pv_pos[bi][0] <= t:
                _, u, j = pv_pos[bi]
                pv_chunk(pv_states[u], j)
                bi += 1
            if t == FFN_UP_AT:
                ffn_up(it)
            if t == FFN_DOWN_AT:
                ffn_down(it)
        assert bi == len(pv_pos) and FFN_UP_AT < FFN_DOWN_AT < NB * NC
        return carry

    for c in late_copies:
        c.wait()
    lax.fori_loop(0, NIT, attn_body, 0)

    assert (NC // PV_PER_PIECE) * TP <= S - TQ
    last = PVState(unit_of(jnp.int32(NIT - 1), NB - 1), (NB - 1) % 2)
    for j in range(S // TP):
        for c in range(min(NC, j * PV_PER_PIECE), min(NC, (j + 1) * PV_PER_PIECE)):
            pv_chunk(last, c)
        rows = slice(j * TP, (j + 1) * TP)
        o = ot_ref[:, rows].T.astype(bf16)
        y = y_ref[rows, :] + jnp.dot(o, wo_ref[...], preferred_element_type=f32)
        o_ref[rows, :] = y.astype(o_ref.dtype)
        drows = pl.ds(j * TP, TP)
        pltpu.make_async_copy(o_ref.at[drows, :], o_hbm.at[drows, :], sem.at[SEM_OUT]).start()
    pltpu.make_async_copy(o_ref, o_hbm, sem.at[SEM_OUT]).wait()


@jax.jit
def pallas_parallel_sum__softmax_full_mha__swiglu_ffn__prompt_kernel(
    A_x: jax.Array,
    A_wqkv: jax.Array,
    A_wo: jax.Array,
    B_x: jax.Array,
    B_w_gate: jax.Array,
    B_w_up: jax.Array,
    B_w_down: jax.Array,
):
    del B_x
    bf16 = jnp.bfloat16
    out = pl.pallas_call(
        _kernel,
        out_shape=jax.ShapeDtypeStruct((S, D), A_x.dtype),
        in_specs=[pl.BlockSpec(memory_space=pl.ANY)] * 6,
        out_specs=pl.BlockSpec(memory_space=pl.ANY),
        scratch_shapes=[
            pltpu.VMEM((S, D), bf16),
            pltpu.VMEM((D, 3 * D), bf16),
            pltpu.VMEM((D, D), bf16),
            pltpu.VMEM((D, F), bf16),
            pltpu.VMEM((D, F), bf16),
            pltpu.VMEM((F, D), bf16),
            pltpu.VMEM((S, D), bf16),
            pltpu.VMEM((D, D), jnp.uint32),
            pltpu.VMEM((S, D), bf16),
            pltpu.VMEM((NKB, S // 2, LANES), jnp.uint32),
            pltpu.VMEM((H, LANES // 2, S), jnp.uint32),
            pltpu.VMEM((H, VROWS, S), jnp.float32),
            pltpu.VMEM((2, S, TQ), jnp.float32),
            pltpu.VMEM((2, 8, TQ), jnp.float32),
            pltpu.VMEM((D, S), jnp.float32),
            pltpu.VMEM((TF // 2, F), jnp.uint32),
            pltpu.VMEM((S, D), jnp.float32),
            pltpu.SemaphoreType.DMA((NSEM,)),
        ],
        compiler_params=pltpu.CompilerParams(vmem_limit_bytes=100 * 2**20),
    )(A_x.reshape(S, D), A_wqkv, A_wo, B_w_gate, B_w_up, B_w_down)
    return out.reshape(1, S, D)
```
